```python
import os as _os
_os.environ.setdefault("JAX_PLATFORMS", "cpu")
import jax
import jax.numpy as jnp

def _softmax(x, axis=-1):
    return jax.nn.softmax(x, axis=axis)
def _gelu(x):
    return jax.nn.gelu(x, approximate=True)
def _silu(x):
    return jax.nn.silu(x)
def _sigmoid(x):
    return jax.nn.sigmoid(x)
def _layernorm(x, axis=-1, eps=1e-5):
    m = jnp.mean(x, axis=axis, keepdims=True)
    v = jnp.var(x, axis=axis, keepdims=True)
    return (x - m) / jnp.sqrt(v + eps)
def _scatter_add(tgt, idx, src, axis=0):
    return tgt.at[idx].add(src)
def _segment_sum(src, seg, n):
    return jax.ops.segment_sum(src, seg, n)
class _Rng:
    def __init__(self, key):
        self._k = key
    def _next(self):
        self._k, sub = jax.random.split(self._k)
        return sub
    def normal(self, shape):
        return jax.random.normal(self._next(), shape, dtype=jnp.bfloat16)
    def randint(self, lo, hi, shape):
        return jax.random.randint(self._next(), shape, lo, hi, dtype=jnp.int32)
    def uniform(self, shape, lo=0.0, hi=1.0):
        return jax.random.uniform(self._next(), shape, jnp.bfloat16, lo, hi)
    def permutation(self, n):
        return jax.random.permutation(self._next(), n)


kernel_name = 'gated_mix__mha_block__mixer_s_mlp__prompt'

def setup_inputs():
    _rng = _Rng(jax.random.key(int.from_bytes(__import__("os").urandom(4), "little")))
    _w = (lambda a: (lambda t: t.astype(jnp.bfloat16) if jnp.issubdtype(t.dtype, jnp.floating) else t)(jnp.asarray(a)))
    def _A_setup():
        B, S, D, H = 1, 2048, 512, 32
        return {
            "x": _w((lambda *s: _rng.normal(s) * 0.05)(B, S, D)),
            "wqkv": _w((lambda *s: _rng.normal(s) * 0.8)(D, 3 * D)),
            "wo": _w((lambda *s: _rng.normal(s) * 0.05)(D, D)),
        }
    _A_in = _A_setup()

    def _B_setup():
        B, S, D, F = 1, 2048, 512, 1792
        return {
            "x":  _w((lambda *s: _rng.normal(s) * 0.05)(B, S, D)),
            "w1": _w((lambda *s: _rng.normal(s) * 0.2)(D, D) * (D ** -0.5)),
            "w2": _w((lambda *s: _rng.normal(s) * 0.2)(D, D) * (D ** -0.5)),
            "w3": _w((lambda *s: _rng.normal(s) * 0.2)(D, F) * (D ** -0.5)),
            "w4": _w((lambda *s: _rng.normal(s) * 0.2)(F, D) * (F ** -0.5)),
        }
    _B_in = _B_setup()

    return {
        "A_x": _A_in["x"],
        "A_wqkv": _A_in["wqkv"],
        "A_wo": _A_in["wo"],
        "B_x": _B_in["x"],
        "B_w1": _B_in["w1"],
        "B_w2": _B_in["w2"],
        "B_w3": _B_in["w3"],
        "B_w4": _B_in["w4"],
        "gate_w": _w((lambda *s: _rng.normal(s) * 0.05)(512) * 16.0),
    }

def reference(A_x, A_wqkv, A_wo, B_x, B_w1, B_w2, B_w3, B_w4, gate_w):
    def _A_ref(x, wqkv, wo):
        B, S, D = x.shape
        H = 32
        Dh = D // H
        qkv = (lambda x, *d: x.transpose(*d))((x @ wqkv).reshape(B, S, 3, H, Dh), 2, 0, 3, 1, 4)
        q, k, v = qkv[0], qkv[1], qkv[2]
        scores = jnp.einsum("bhqd,bhkd->bhqk", q, k) * (Dh ** -0.5)
        p = _softmax(scores, axis=-1)
        o = jnp.einsum("bhqk,bhkd->bhqd", p, v)
        return (lambda x, *d: x.transpose(*d))(o, 0, 2, 1, 3).reshape(B, S, D) @ wo

    def _B_ref(x, w1, w2, w3, w4):
        B, S, D = x.shape
        h = _gelu(_layernorm(x, axis=-1) @ w1)
        c = D // 4
        g0 = jnp.pad(h[:, :, 0*c:1*c], ((0, 0), (1, 0), (0, 0)))[:, :S, :]
        g1 = jnp.pad(h[:, :, 1*c:2*c], ((0, 0), (0, 1), (0, 0)))[:, 1:, :]
        g2 = jnp.pad(h[:, :, 2*c:3*c], ((0, 0), (2, 0), (0, 0)))[:, :S, :]
        g3 = jnp.pad(h[:, :, 3*c:   ], ((0, 0), (0, 2), (0, 0)))[:, 2:, :]
        hs = jnp.concatenate([g0, g1, g2, g3], axis=-1) @ w2
        x1 = x + hs
        h2 = _gelu(_layernorm(x1, axis=-1) @ w3) @ w4
        return x1 + h2

    x = A_x
    g = _sigmoid((x * gate_w).sum(-1, keepdims=True))
    a = _A_ref(x, A_wqkv, A_wo)
    b = _B_ref(x, B_w1, B_w2, B_w3, B_w4)
    return g * a + (1 - g) * b
```

```python
import functools
import math

import jax
import jax.numpy as jnp
import jax.experimental.pallas as pl
import jax.experimental.pallas.tpu as pltpu

S = 2048
D = 512
H = 32
DH = 16
F = 1792
NG = D // 128
HPG = 128 // DH
TQ = 256
PB = 256
PAD = 8
EPS = 1e-5
QSCALE = (DH ** -0.5) * math.log2(math.e)


def _gelu(x):
    c = math.sqrt(2.0 / math.pi)
    return 0.5 * x * (1.0 + jnp.tanh(c * (x + 0.044715 * (x * x * x))))


def _layernorm(x):
    m = jnp.mean(x, axis=-1, keepdims=True)
    xc = x - m
    v = jnp.mean(xc * xc, axis=-1, keepdims=True)
    return xc * jax.lax.rsqrt(v + EPS)


def _kernel(ax_ref, wqkv_ref, wo_ref, w1_ref, w2_ref, w3_ref, w4_ref, gw_ref,
            o_ref, k_scr, qt_scr, vt_scr, h_scr, ot_scr):
    i = pl.program_id(0)
    f32 = jnp.float32
    bf16 = jnp.bfloat16

    @pl.when(i == 0)
    def _():
        h_scr[0:PAD, :] = jnp.zeros((PAD, D), f32)
        h_scr[PAD + S:PAD + S + PAD, :] = jnp.zeros((PAD, D), f32)

        def proj(b, carry):
            r0 = pl.multiple_of(b * PB, PB)
            x = ax_ref[pl.ds(r0, PB), :]
            qkv = jnp.dot(x, wqkv_ref[...], preferred_element_type=f32)
            qt = (qkv[:, 0:D] * QSCALE).T.astype(bf16)
            vt = qkv[:, 2 * D:3 * D].T.astype(bf16)
            k = qkv[:, D:2 * D].astype(bf16)
            for g in range(NG):
                k_scr[g, pl.ds(r0, PB), :] = k[:, g * 128:(g + 1) * 128]
            qt_scr[b] = qt
            vt_scr[b] = vt
            xb = x.astype(f32)
            h = _gelu(jnp.dot(_layernorm(xb).astype(bf16), w1_ref[...], preferred_element_type=f32))
            h_scr[pl.ds(PAD + r0, PB), :] = h
            return carry

        jax.lax.fori_loop(0, S // PB, proj, 0)

    row_head = jax.lax.broadcasted_iota(jnp.int32, (128, TQ), 0) // DH

    def head(h, carry):
        g = h // HPG
        j = h % HPG
        qg = qt_scr[i, pl.ds(pl.multiple_of(g * 128, 128), 128), :]
        w = jnp.where(row_head == j, qg, jnp.zeros_like(qg))
        s = jnp.dot(k_scr[g], w, preferred_element_type=f32)
        m = jnp.max(s, axis=0, keepdims=True)
        p = jnp.exp2(s - m)
        l = jnp.sum(p, axis=0, keepdims=True)
        pb = p.astype(bf16)
        r = pl.ds(pl.multiple_of(h * DH, DH), DH)
        o = jnp.zeros((DH, TQ), f32)
        for b in range(S // PB):
            o = o + jnp.dot(vt_scr[b, r, :], pb[b * PB:(b + 1) * PB, :], preferred_element_type=f32)
        ot_scr[r, :] = o / l
        return carry

    jax.lax.fori_loop(0, H, head, 0)

    r0 = pl.multiple_of(i * TQ, TQ)
    o_att = ot_scr[...].T.astype(bf16)
    a = jnp.dot(o_att, wo_ref[...], preferred_element_type=f32)

    c = D // 4
    hw = h_scr[pl.ds(r0, TQ + 2 * PAD), :]
    hs_in = jnp.concatenate([
        hw[PAD - 1:PAD - 1 + TQ, 0 * c:1 * c],
        hw[PAD + 1:PAD + 1 + TQ, 1 * c:2 * c],
        hw[PAD - 2:PAD - 2 + TQ, 2 * c:3 * c],
        hw[PAD + 2:PAD + 2 + TQ, 3 * c:4 * c],
    ], axis=-1).astype(bf16)
    xb = ax_ref[pl.ds(r0, TQ), :].astype(f32)
    x1 = xb + jnp.dot(hs_in, w2_ref[...], preferred_element_type=f32)
    t = _gelu(jnp.dot(_layernorm(x1).astype(bf16), w3_ref[...], preferred_element_type=f32))
    bb = x1 + jnp.dot(t.astype(bf16), w4_ref[...], preferred_element_type=f32)

    xa = ax_ref[pl.ds(r0, TQ), :].astype(f32)
    gate = jax.nn.sigmoid(jnp.sum(xa * gw_ref[...].astype(f32), axis=-1, keepdims=True))
    o_ref[...] = (gate * a + (1.0 - gate) * bb).astype(o_ref.dtype)


@jax.jit
def pallas_gated_mix__mha_block__mixer_s_mlp__prompt_kernel(
    A_x: jax.Array,
    A_wqkv: jax.Array,
    A_wo: jax.Array,
    B_x: jax.Array,
    B_w1: jax.Array,
    B_w2: jax.Array,
    B_w3: jax.Array,
    B_w4: jax.Array,
    gate_w: jax.Array,
):
    assert PB == TQ
    ax = A_x.reshape(S, D)
    gw = gate_w.reshape(1, D)

    def full(shape):
        return pl.BlockSpec(shape, lambda i: (0,) * len(shape))

    out = pl.pallas_call(
        _kernel,
        grid=(S // TQ,),
        in_specs=[full((S, D)), full((D, 3 * D)), full((D, D)), full((D, D)),
                  full((D, D)), full((D, F)), full((F, D)), full((1, D))],
        out_specs=pl.BlockSpec((TQ, D), lambda i: (i, 0)),
        out_shape=jax.ShapeDtypeStruct((S, D), jnp.bfloat16),
        scratch_shapes=[
            pltpu.VMEM((NG, S, 128), jnp.bfloat16),
            pltpu.VMEM((S // PB, D, PB), jnp.bfloat16),
            pltpu.VMEM((S // PB, D, PB), jnp.bfloat16),
            pltpu.VMEM((S + 2 * PAD, D), jnp.float32),
            pltpu.VMEM((D, TQ), jnp.float32),
        ],
        compiler_params=pltpu.CompilerParams(
            dimension_semantics=("arbitrary",),
            vmem_limit_bytes=100 * 1024 * 1024),
    )(ax, A_wqkv, A_wo, B_w1, B_w2, B_w3, B_w4, gw)
    return out.reshape(1, S, D)
```

```python
import functools
import math

import jax
import jax.numpy as jnp
import jax.experimental.pallas as pl
import jax.experimental.pallas.tpu as pltpu

S = 2048
D = 512
H = 32
DH = 16
F = 1792
NG = D // 128
HPG = 128 // DH
TQ = 256
NB = S // TQ
CK = 128
NC = S // CK
LA = 4
FC = 256
PAD = 8
EPS = 1e-5
QSCALE = (DH ** -0.5) * math.log2(math.e)
L_MIN = 2.0 ** -40
L_MAX = 1.0e6

f32 = jnp.float32
bf16 = jnp.bfloat16
_NT = (((1,), (1,)), ((), ()))


def _gelu(x):
    c = math.sqrt(2.0 / math.pi)
    return 0.5 * x * (1.0 + jnp.tanh(c * (x + 0.044715 * (x * x * x))))


def _layernorm(x):
    m = jnp.mean(x, axis=-1, keepdims=True)
    xc = x - m
    v = jnp.mean(xc * xc, axis=-1, keepdims=True)
    return xc * jax.lax.rsqrt(v + EPS)


def _dot(a, b):
    return jnp.dot(a, b, preferred_element_type=f32)


def _dot_nt(a, b):
    return jax.lax.dot_general(a, b, _NT, preferred_element_type=f32)


def _masked_q(qh, j):
    parts = []
    if j > 0:
        parts.append(jnp.zeros((j * DH, TQ), bf16))
    parts.append(qh)
    if j < HPG - 1:
        parts.append(jnp.zeros(((HPG - 1 - j) * DH, TQ), bf16))
    return jnp.concatenate(parts, axis=0)


def _kernel(x_hbm, wqkv_hbm, wo_hbm, w1_hbm, w2_hbm, w3_hbm, w4_hbm, gw_ref,
            o_ref,
            x_v, wqkv_v, wo_v, w1_v, w2_v, w3_v, w4_v, sems,
            wqt_scr, wvt_scr, k_scr, qt_scr, vt_scr, h_scr, ot_scr, l_scr, qn_scr, kn_scr):
    i = pl.program_id(0)

    def copies():
        pairs = [(wqkv_hbm, wqkv_v), (x_hbm, x_v), (w1_hbm, w1_v), (w2_hbm, w2_v),
                 (wo_hbm, wo_v), (w3_hbm, w3_v), (w4_hbm, w4_v)]
        return [pltpu.make_async_copy(s, d, sems.at[n]) for n, (s, d) in enumerate(pairs)]

    @pl.when(i == 0)
    def _():
        cps = copies()
        for cp in cps:
            cp.start()
        h_scr[0:PAD, :] = jnp.zeros((PAD, D), f32)
        h_scr[PAD + S:PAD + S + PAD, :] = jnp.zeros((PAD, D), f32)
        cps[0].wait()
        wqt_scr[...] = wqkv_v[:, 0:D].astype(f32).T.astype(bf16)
        wvt_scr[...] = wqkv_v[:, 2 * D:3 * D].astype(f32).T.astype(bf16)
        cps[1].wait()
        cps[2].wait()
        gsel = (jax.lax.broadcasted_iota(jnp.int32, (H, D), 1) // DH
                == jax.lax.broadcasted_iota(jnp.int32, (H, D), 0))
        gmat = jnp.where(gsel, 1.0, 0.0).astype(bf16)

        def proj(b, kn_max):
            r0 = pl.multiple_of(b * TQ, TQ)
            x = x_v[pl.ds(r0, TQ), :]
            ln = _layernorm(x.astype(f32)).astype(bf16)
            k = _dot(x, wqkv_v[:, D:2 * D]).astype(bf16)
            qt = (_dot_nt(wqt_scr[...], x) * QSCALE).astype(bf16)
            vt = _dot_nt(wvt_scr[...], x).astype(bf16)
            u = _dot(ln, w1_v[...])
            for g in range(NG):
                k_scr[g, pl.ds(r0, TQ), :] = k[:, g * 128:(g + 1) * 128]
            qt_scr[b] = qt
            vt_scr[b] = vt
            h_scr[pl.ds(PAD + r0, TQ), :] = _gelu(u)
            kf = k.astype(f32)
            qf = qt.astype(f32)
            qn_scr[b] = _dot(gmat, (qf * qf).astype(bf16))
            kn = _dot_nt(gmat, (kf * kf).astype(bf16))
            return jnp.maximum(kn_max, kn)

        kn_max = jax.lax.fori_loop(0, NB, proj, jnp.zeros((H, TQ), f32))
        kn_scr[...] = jnp.broadcast_to(jnp.max(kn_max, axis=1, keepdims=True), (H, TQ))
        for cp in cps[3:]:
            cp.wait()

    mb = jnp.sqrt(qn_scr[i] * kn_scr[...]) * 1.01

    def vt_chunk(h, c):
        per = TQ // CK
        return vt_scr[c // per, h * DH:(h + 1) * DH, (c % per) * CK:(c % per + 1) * CK]

    items = [(h, c) for h in range(H) for c in range(NC)]
    ws = {}

    def qk(t):
        h, c = items[t]
        if c == 0:
            ws[h] = _masked_q(qt_scr[i, h * DH:(h + 1) * DH, :], h % HPG)
        return _dot(k_scr[h // HPG, c * CK:(c + 1) * CK, :], ws[h])

    pend = {t: qk(t) for t in range(LA)}
    for t, (h, c) in enumerate(items):
        if c == 0:
            m = mb[h:h + 1, :]
            l8 = jnp.zeros((8, TQ), f32)
            o = jnp.zeros((DH, TQ), f32)
        if t + LA < len(items):
            pend[t + LA] = qk(t + LA)
        p = jnp.exp2(pend.pop(t) - m)
        l8 = l8 + jnp.sum(p.reshape(CK // 8, 8, TQ), axis=0)
        o = o + _dot(vt_chunk(h, c), p.astype(bf16))
        if c == NC - 1:
            l = jnp.sum(l8, axis=0, keepdims=True)
            l_scr[h:h + 1, :] = l
            ot_scr[h * DH:(h + 1) * DH, :] = o / l

    l_all = l_scr[...]
    safe = jnp.logical_and(jnp.min(l_all) >= L_MIN, jnp.max(l_all) <= L_MAX)

    @pl.when(jnp.logical_not(safe))
    def _():
        row_head = jax.lax.broadcasted_iota(jnp.int32, (128, TQ), 0) // DH

        def head(h, carry):
            g = h // HPG
            qg = qt_scr[i, pl.ds(pl.multiple_of(g * 128, 128), 128), :]
            w = jnp.where(row_head == h % HPG, qg, jnp.zeros_like(qg))
            s = _dot(k_scr[g], w)
            p = jnp.exp2(s - jnp.max(s, axis=0, keepdims=True))
            l = jnp.sum(p, axis=0, keepdims=True)
            pb = p.astype(bf16)
            r = pl.ds(pl.multiple_of(h * DH, DH), DH)
            o = jnp.zeros((DH, TQ), f32)
            for b in range(NB):
                o = o + _dot(vt_scr[b, r, :], pb[b * TQ:(b + 1) * TQ, :])
            ot_scr[r, :] = o / l
            return carry

        jax.lax.fori_loop(0, H, head, 0)

    r0 = pl.multiple_of(i * TQ, TQ)
    c4 = D // 4
    hw = h_scr[pl.ds(r0, TQ + 2 * PAD), :]
    hs_in = jnp.concatenate([
        hw[PAD - 1:PAD - 1 + TQ, 0 * c4:1 * c4],
        hw[PAD + 1:PAD + 1 + TQ, 1 * c4:2 * c4],
        hw[PAD - 2:PAD - 2 + TQ, 2 * c4:3 * c4],
        hw[PAD + 2:PAD + 2 + TQ, 3 * c4:4 * c4],
    ], axis=-1).astype(bf16)
    xf = x_v[pl.ds(r0, TQ), :].astype(f32)
    x1 = xf + _dot(hs_in, w2_v[...])
    o_att = ot_scr[...].T.astype(bf16)
    a = _dot(o_att, wo_v[...])
    ln1 = _layernorm(x1).astype(bf16)
    nf = F // FC
    u_next = _dot(ln1, w3_v[:, 0:FC])
    bb = x1
    for c in range(nf):
        u = u_next
        if c + 1 < nf:
            u_next = _dot(ln1, w3_v[:, (c + 1) * FC:(c + 2) * FC])
        bb = bb + _dot(_gelu(u).astype(bf16), w4_v[c * FC:(c + 1) * FC, :])

    gate = jax.nn.sigmoid(jnp.sum(xf * gw_ref[...].astype(f32), axis=-1, keepdims=True))
    o_ref[...] = (gate * a + (1.0 - gate) * bb).astype(o_ref.dtype)


@jax.jit
def pallas_gated_mix__mha_block__mixer_s_mlp__prompt_kernel(
    A_x: jax.Array,
    A_wqkv: jax.Array,
    A_wo: jax.Array,
    B_x: jax.Array,
    B_w1: jax.Array,
    B_w2: jax.Array,
    B_w3: jax.Array,
    B_w4: jax.Array,
    gate_w: jax.Array,
):
    ax = A_x.reshape(S, D)
    gw = gate_w.reshape(1, D)
    hbm = pl.BlockSpec(memory_space=pl.ANY)
    out = pl.pallas_call(
        _kernel,
        grid=(NB,),
        in_specs=[hbm] * 7 + [pl.BlockSpec((1, D), lambda i: (0, 0))],
        out_specs=pl.BlockSpec((TQ, D), lambda i: (i, 0)),
        out_shape=jax.ShapeDtypeStruct((S, D), bf16),
        scratch_shapes=[
            pltpu.VMEM((S, D), bf16),
            pltpu.VMEM((D, 3 * D), bf16),
            pltpu.VMEM((D, D), bf16),
            pltpu.VMEM((D, D), bf16),
            pltpu.VMEM((D, D), bf16),
            pltpu.VMEM((D, F), bf16),
            pltpu.VMEM((F, D), bf16),
            pltpu.SemaphoreType.DMA((7,)),
            pltpu.VMEM((D, D), bf16),
            pltpu.VMEM((D, D), bf16),
            pltpu.VMEM((NG, S, 128), bf16),
            pltpu.VMEM((NB, D, TQ), bf16),
            pltpu.VMEM((NB, D, TQ), bf16),
            pltpu.VMEM((S + 2 * PAD, D), f32),
            pltpu.VMEM((D, TQ), f32),
            pltpu.VMEM((H, TQ), f32),
            pltpu.VMEM((NB, H, TQ), f32),
            pltpu.VMEM((H, TQ), f32),
        ],
        compiler_params=pltpu.CompilerParams(
            dimension_semantics=("arbitrary",),
            vmem_limit_bytes=100 * 1024 * 1024),
    )(ax, A_wqkv, A_wo, B_w1, B_w2, B_w3, B_w4, gw)
    return out.reshape(1, S, D)
```

```python
import functools
import math

import jax
import jax.numpy as jnp
import jax.experimental.pallas as pl
import jax.experimental.pallas.tpu as pltpu

S = 2048
D = 512
H = 32
DH = 16
F = 1792
NG = D // 128
HPG = 128 // DH
TQ = 256
NB = S // TQ
CK = 128
NC = S // CK
LA = 4
FC = 256
PUNR = 2
PAD = 8
EPS = 1e-5
QSCALE = (DH ** -0.5) * math.log2(math.e)
L_MIN = 2.0 ** -40
L_MAX = 1.0e6

f32 = jnp.float32
bf16 = jnp.bfloat16
_NT = (((1,), (1,)), ((), ()))


def _gelu(x):
    c = math.sqrt(2.0 / math.pi)
    return 0.5 * x * (1.0 + jnp.tanh(c * (x + 0.044715 * (x * x * x))))


def _layernorm(x):
    m = jnp.mean(x, axis=-1, keepdims=True)
    xc = x - m
    v = jnp.mean(xc * xc, axis=-1, keepdims=True)
    return xc * jax.lax.rsqrt(v + EPS)


def _dot(a, b):
    return jnp.dot(a, b, preferred_element_type=f32)


def _dot_nt(a, b):
    return jax.lax.dot_general(a, b, _NT, preferred_element_type=f32)


def _masked_q(qh, j):
    parts = []
    if j > 0:
        parts.append(jnp.zeros((j * DH, TQ), bf16))
    parts.append(qh)
    if j < HPG - 1:
        parts.append(jnp.zeros(((HPG - 1 - j) * DH, TQ), bf16))
    return jnp.concatenate(parts, axis=0)


def _kernel(x_hbm, wqkv_hbm, wo_hbm, w1_hbm, w2_hbm, w3_hbm, w4_hbm, gw_ref,
            o_ref,
            x_v, wqkv_v, wo_v, w1_v, w2_v, w3_v, w4_v, sems, xsems,
            wqt_scr, wvt_scr, k_scr, qt_scr, vt_scr, h_scr, ot_scr, l_scr, qn_scr, kn_scr,
            gb_scr, gate_scr):
    i = pl.program_id(0)

    def copies():
        pairs = [(wqkv_hbm.at[:, 0:D], wqkv_v.at[:, 0:D]),
                 (wqkv_hbm.at[:, 2 * D:3 * D], wqkv_v.at[:, 2 * D:3 * D]),
                 (wqkv_hbm.at[:, D:2 * D], wqkv_v.at[:, D:2 * D]),
                 (w1_hbm, w1_v),
                 (w2_hbm, w2_v), (wo_hbm, wo_v), (w3_hbm, w3_v), (w4_hbm, w4_v)]
        return [pltpu.make_async_copy(s, d, sems.at[n]) for n, (s, d) in enumerate(pairs)]

    def x_copy(b):
        rows = pl.ds(pl.multiple_of(b * TQ, TQ), TQ)
        return pltpu.make_async_copy(x_hbm.at[rows], x_v.at[rows], xsems.at[b])

    @pl.when(i == 0)
    def _():
        cps = copies()
        cps[0].start()
        cps[1].start()
        cps[2].start()
        x_copy(0).start()
        cps[3].start()
        h_scr[0:PAD, :] = jnp.zeros((PAD, D), f32)
        h_scr[PAD + S:PAD + S + PAD, :] = jnp.zeros((PAD, D), f32)
        gsel = (jax.lax.broadcasted_iota(jnp.int32, (H, D), 1) // DH
                == jax.lax.broadcasted_iota(jnp.int32, (H, D), 0))
        gmat = jnp.where(gsel, 1.0, 0.0).astype(bf16)

        def proj(b, kn_max):
            r0 = pl.multiple_of(b * TQ, TQ)
            x_copy(b).wait()
            x = x_v[pl.ds(r0, TQ), :]
            ln = _layernorm(x.astype(f32)).astype(bf16)
            k = _dot(x, wqkv_v[:, D:2 * D]).astype(bf16)
            qt = (_dot_nt(wqt_scr[...], x) * QSCALE).astype(bf16)
            vt = _dot_nt(wvt_scr[...], x).astype(bf16)
            u = _dot(ln, w1_v[...])
            for g in range(NG):
                k_scr[g, pl.ds(r0, TQ), :] = k[:, g * 128:(g + 1) * 128]
            qt_scr[b] = qt
            vt_scr[b] = vt
            h_scr[pl.ds(PAD + r0, TQ), :] = _gelu(u)
            kf = k.astype(f32)
            qf = qt.astype(f32)
            qn_scr[b] = _dot(gmat, (qf * qf).astype(bf16))
            kn = _dot_nt(gmat, (kf * kf).astype(bf16))
            return jnp.maximum(kn_max, kn)

        cps[0].wait()
        for b in range(1, NB):
            x_copy(b).start()
        wqt_scr[...] = wqkv_v[:, 0:D].astype(f32).T.astype(bf16)
        cps[1].wait()
        wvt_scr[...] = wqkv_v[:, 2 * D:3 * D].astype(f32).T.astype(bf16)
        cps[2].wait()
        cps[3].wait()
        for cp in cps[4:]:
            cp.start()

        def proj_u(bb, kn_max):
            for uu in range(PUNR):
                kn_max = proj(bb * PUNR + uu, kn_max)
            return kn_max

        kn_max = jax.lax.fori_loop(0, NB // PUNR, proj_u, jnp.zeros((H, TQ), f32))
        kn_scr[...] = jnp.broadcast_to(jnp.max(kn_max, axis=1, keepdims=True), (H, TQ))
        for cp in cps[4:]:
            cp.wait()

    mb = jnp.sqrt(qn_scr[i] * kn_scr[...]) * 1.01

    def vt_chunk(h, c):
        per = TQ // CK
        return vt_scr[c // per, h * DH:(h + 1) * DH, (c % per) * CK:(c % per + 1) * CK]

    items = [(h, c) for h in range(H) for c in range(NC)]
    ws = {}

    def qk(t):
        h, c = items[t]
        if c == 0:
            ws[h] = _masked_q(qt_scr[i, h * DH:(h + 1) * DH, :], h % HPG)
        return _dot(k_scr[h // HPG, c * CK:(c + 1) * CK, :], ws[h])

    pend = {t: qk(t) for t in range(LA)}
    for t, (h, c) in enumerate(items):
        if c == 0:
            m = mb[h:h + 1, :]
            l8 = jnp.zeros((8, TQ), f32)
            o = jnp.zeros((DH, TQ), f32)
        if t + LA < len(items):
            pend[t + LA] = qk(t + LA)
        p = jnp.exp2(pend.pop(t) - m)
        l8 = l8 + jnp.sum(p.reshape(CK // 8, 8, TQ), axis=0)
        o = o + _dot(vt_chunk(h, c), p.astype(bf16))
        if c == NC - 1:
            l = jnp.sum(l8, axis=0, keepdims=True)
            l_scr[h:h + 1, :] = l
            ot_scr[h * DH:(h + 1) * DH, :] = o / l

    r0 = pl.multiple_of(i * TQ, TQ)
    c4 = D // 4
    hw = h_scr[pl.ds(r0, TQ + 2 * PAD), :]
    hs_in = jnp.concatenate([
        hw[PAD - 1:PAD - 1 + TQ, 0 * c4:1 * c4],
        hw[PAD + 1:PAD + 1 + TQ, 1 * c4:2 * c4],
        hw[PAD - 2:PAD - 2 + TQ, 2 * c4:3 * c4],
        hw[PAD + 2:PAD + 2 + TQ, 3 * c4:4 * c4],
    ], axis=-1).astype(bf16)
    xf = x_v[pl.ds(r0, TQ), :].astype(f32)
    x1 = xf + _dot(hs_in, w2_v[...])
    a = _dot(ot_scr[...].T.astype(bf16), wo_v[...])
    ln1 = _layernorm(x1).astype(bf16)
    nf = F // FC
    u_next = _dot(ln1, w3_v[:, 0:FC])
    bb = x1
    for c in range(nf):
        u = u_next
        if c + 1 < nf:
            u_next = _dot(ln1, w3_v[:, (c + 1) * FC:(c + 2) * FC])
        bb = bb + _dot(_gelu(u).astype(bf16), w4_v[c * FC:(c + 1) * FC, :])

    gate = jax.nn.sigmoid(jnp.sum(xf * gw_ref[...].astype(f32).reshape(1, D), axis=-1, keepdims=True))
    gb = (1.0 - gate) * bb
    gb_scr[...] = gb
    gate_scr[...] = gate
    o_ref[...] = (gate * a + gb).astype(o_ref.dtype)

    l_all = l_scr[...]
    safe = jnp.logical_and(jnp.min(l_all) >= L_MIN, jnp.max(l_all) <= L_MAX)

    @pl.when(jnp.logical_not(safe))
    def _():
        row_head = jax.lax.broadcasted_iota(jnp.int32, (128, TQ), 0) // DH

        def head(h, carry):
            g = h // HPG
            qg = qt_scr[i, pl.ds(pl.multiple_of(g * 128, 128), 128), :]
            w = jnp.where(row_head == h % HPG, qg, jnp.zeros_like(qg))
            s = _dot(k_scr[g], w)
            p = jnp.exp2(s - jnp.max(s, axis=0, keepdims=True))
            l = jnp.sum(p, axis=0, keepdims=True)
            pb = p.astype(bf16)
            r = pl.ds(pl.multiple_of(h * DH, DH), DH)
            o = jnp.zeros((DH, TQ), f32)
            for b in range(NB):
                o = o + _dot(vt_scr[b, r, :], pb[b * TQ:(b + 1) * TQ, :])
            ot_scr[r, :] = o / l
            return carry

        jax.lax.fori_loop(0, H, head, 0)
        a2 = _dot(ot_scr[...].T.astype(bf16), wo_v[...])
        o_ref[...] = (gate_scr[...] * a2 + gb_scr[...]).astype(o_ref.dtype)


@jax.jit
def pallas_gated_mix__mha_block__mixer_s_mlp__prompt_kernel(
    A_x: jax.Array,
    A_wqkv: jax.Array,
    A_wo: jax.Array,
    B_x: jax.Array,
    B_w1: jax.Array,
    B_w2: jax.Array,
    B_w3: jax.Array,
    B_w4: jax.Array,
    gate_w: jax.Array,
):
    ax = A_x.reshape(S, D)
    hbm = pl.BlockSpec(memory_space=pl.ANY)
    out = pl.pallas_call(
        _kernel,
        grid=(NB,),
        in_specs=[hbm] * 7 + [pl.BlockSpec((D,), lambda i: (0,))],
        out_specs=pl.BlockSpec((TQ, D), lambda i: (i, 0)),
        out_shape=jax.ShapeDtypeStruct((S, D), bf16),
        scratch_shapes=[
            pltpu.VMEM((S, D), bf16),
            pltpu.VMEM((D, 3 * D), bf16),
            pltpu.VMEM((D, D), bf16),
            pltpu.VMEM((D, D), bf16),
            pltpu.VMEM((D, D), bf16),
            pltpu.VMEM((D, F), bf16),
            pltpu.VMEM((F, D), bf16),
            pltpu.SemaphoreType.DMA((8,)),
            pltpu.SemaphoreType.DMA((NB,)),
            pltpu.VMEM((D, D), bf16),
            pltpu.VMEM((D, D), bf16),
            pltpu.VMEM((NG, S, 128), bf16),
            pltpu.VMEM((NB, D, TQ), bf16),
            pltpu.VMEM((NB, D, TQ), bf16),
            pltpu.VMEM((S + 2 * PAD, D), f32),
            pltpu.VMEM((D, TQ), f32),
            pltpu.VMEM((H, TQ), f32),
            pltpu.VMEM((NB, H, TQ), f32),
            pltpu.VMEM((H, TQ), f32),
            pltpu.VMEM((TQ, D), f32),
            pltpu.VMEM((TQ, 1), f32),
        ],
        compiler_params=pltpu.CompilerParams(
            dimension_semantics=("arbitrary",),
            vmem_limit_bytes=100 * 1024 * 1024),
    )(ax, A_wqkv, A_wo, B_w1, B_w2, B_w3, B_w4, gate_w)
    return out.reshape(1, S, D)
```

```python
import math

import jax
import jax.numpy as jnp
import jax.experimental.pallas as pl
import jax.experimental.pallas.tpu as pltpu

S = 2048
D = 512
H = 32
DH = 16
F = 1792
NG = D // 128
HPG = 128 // DH
TQ = 256
NB = S // TQ
CK = 128
NC = S // CK
LA = 4
FC = 256
PUNR = 2
PAD = 8
EPS = 1e-5
QSCALE = (DH ** -0.5) * math.log2(math.e)
L_MIN = 2.0 ** -40
L_MAX = 1.0e6

f32 = jnp.float32
bf16 = jnp.bfloat16
_NT = (((1,), (1,)), ((), ()))


def _gelu(x):
    c = math.sqrt(2.0 / math.pi)
    return 0.5 * x * (1.0 + jnp.tanh(c * (x + 0.044715 * (x * x * x))))


def _layernorm(x):
    m = jnp.mean(x, axis=-1, keepdims=True)
    xc = x - m
    v = jnp.mean(xc * xc, axis=-1, keepdims=True)
    return xc * jax.lax.rsqrt(v + EPS)


def _dot(a, b):
    return jnp.dot(a, b, preferred_element_type=f32)


def _dot_nt(a, b):
    return jax.lax.dot_general(a, b, _NT, preferred_element_type=f32)


def _masked_q(qh, j):
    parts = []
    if j > 0:
        parts.append(jnp.zeros((j * DH, TQ), bf16))
    parts.append(qh)
    if j < HPG - 1:
        parts.append(jnp.zeros(((HPG - 1 - j) * DH, TQ), bf16))
    return jnp.concatenate(parts, axis=0)


def _kernel(x_hbm, wqkv_hbm, wo_hbm, w1_hbm, w2_hbm, w3_hbm, w4_hbm, gw_ref,
            o_ref,
            x_v, wqkv_v, wo_v, w1_v, w2_v, w3_v, w4_v, sems, xsems,
            wqt_scr, wvt_scr, k_scr, qt_scr, vt_scr, ot_scr, l_scr, kn_scr,
            gb_scr, gate_scr):
    i = pl.program_id(0)

    def copies():
        pairs = [(wqkv_hbm.at[:, 2 * D:3 * D], wqkv_v.at[:, 2 * D:3 * D]),
                 (wqkv_hbm.at[:, D:2 * D], wqkv_v.at[:, D:2 * D]),
                 (wqkv_hbm.at[:, 0:D], wqkv_v.at[:, 0:D]),
                 (w1_hbm, w1_v), (w2_hbm, w2_v), (wo_hbm, wo_v), (w3_hbm, w3_v), (w4_hbm, w4_v)]
        return [pltpu.make_async_copy(s, d, sems.at[n]) for n, (s, d) in enumerate(pairs)]

    def x_copy(b):
        rows = pl.ds(pl.multiple_of(b * TQ, TQ), TQ)
        return pltpu.make_async_copy(x_hbm.at[rows], x_v.at[rows], xsems.at[b])

    gsel = (jax.lax.broadcasted_iota(jnp.int32, (H, D), 1) // DH
            == jax.lax.broadcasted_iota(jnp.int32, (H, D), 0))
    gmat = jnp.where(gsel, 1.0, 0.0).astype(bf16)

    @pl.when(i == 0)
    def _():
        cps = copies()
        cps[0].start()
        cps[1].start()
        for b in range(PUNR):
            x_copy(b).start()
        x_v[S:S + PAD, :] = jnp.zeros((PAD, D), bf16)

        def proj(b, kn_max):
            r0 = pl.multiple_of(b * TQ, TQ)
            x = x_v[pl.ds(r0, TQ), :]
            k = _dot(x, wqkv_v[:, D:2 * D]).astype(bf16)
            vt = _dot_nt(wvt_scr[...], x).astype(bf16)
            for g in range(NG):
                k_scr[g, pl.ds(r0, TQ), :] = k[:, g * 128:(g + 1) * 128]
            vt_scr[b] = vt
            kf = k.astype(f32)
            kn = _dot_nt(gmat, (kf * kf).astype(bf16))
            return jnp.maximum(kn_max, kn)

        cps[0].wait()
        for b in range(PUNR, NB):
            x_copy(b).start()
        wvt_scr[...] = wqkv_v[:, 2 * D:3 * D].astype(f32).T.astype(bf16)
        cps[1].wait()
        for cp in cps[2:]:
            cp.start()

        def proj_u(bb, kn_max):
            for uu in range(PUNR):
                x_copy(bb * PUNR + uu).wait()
            for uu in range(PUNR):
                kn_max = proj(bb * PUNR + uu, kn_max)
            return kn_max

        kn_max = jax.lax.fori_loop(0, NB // PUNR, proj_u, jnp.zeros((H, TQ), f32))
        kn_scr[...] = jnp.broadcast_to(jnp.max(kn_max, axis=1, keepdims=True), (H, TQ))
        cps[2].wait()
        wqt_scr[...] = wqkv_v[:, 0:D].astype(f32).T.astype(bf16)
        for cp in cps[3:]:
            cp.wait()

    r0 = pl.multiple_of(i * TQ, TQ)
    xq = x_v[pl.ds(r0, TQ), :]
    qt = (_dot_nt(wqt_scr[...], xq) * QSCALE).astype(bf16)
    qt_scr[...] = qt
    rh = pl.multiple_of(jnp.maximum(r0 - PAD, 0), PAD)
    xh = x_v[pl.ds(rh, TQ + 2 * PAD), :].astype(f32)
    hw = _gelu(_dot(_layernorm(xh).astype(bf16), w1_v[...]))
    row = rh + jax.lax.broadcasted_iota(jnp.int32, (TQ + 2 * PAD, 1), 0)
    hw = jnp.where(row < S, hw, 0.0)
    zpad = jnp.zeros((PAD, D), f32)
    hw = jnp.where(i == 0, jnp.concatenate([zpad, hw[0:TQ + PAD, :]], axis=0), hw)
    qf = qt.astype(f32)
    qn = _dot(gmat, (qf * qf).astype(bf16))

    mb = jnp.sqrt(qn * kn_scr[...]) * 1.01

    def vt_chunk(h, c):
        per = TQ // CK
        return vt_scr[c // per, h * DH:(h + 1) * DH, (c % per) * CK:(c % per + 1) * CK]

    items = [(h, c) for h in range(H) for c in range(NC)]
    ws = {}

    def qk(t):
        h, c = items[t]
        if c == 0:
            ws[h] = _masked_q(qt[h * DH:(h + 1) * DH, :], h % HPG)
        return _dot(k_scr[h // HPG, c * CK:(c + 1) * CK, :], ws[h])

    pend = {t: qk(t) for t in range(LA)}
    for t, (h, c) in enumerate(items):
        if c == 0:
            m = mb[h:h + 1, :]
            l8 = jnp.zeros((8, TQ), f32)
            o = jnp.zeros((DH, TQ), f32)
        if t + LA < len(items):
            pend[t + LA] = qk(t + LA)
        p = jnp.exp2(pend.pop(t) - m)
        l8 = l8 + jnp.sum(p.reshape(CK // 8, 8, TQ), axis=0)
        o = o + _dot(vt_chunk(h, c), p.astype(bf16))
        if c == NC - 1:
            l = jnp.sum(l8, axis=0, keepdims=True)
            l_scr[h:h + 1, :] = l
            ot_scr[h * DH:(h + 1) * DH, :] = o / l

    c4 = D // 4
    hs_in = jnp.concatenate([
        hw[PAD - 1:PAD - 1 + TQ, 0 * c4:1 * c4],
        hw[PAD + 1:PAD + 1 + TQ, 1 * c4:2 * c4],
        hw[PAD - 2:PAD - 2 + TQ, 2 * c4:3 * c4],
        hw[PAD + 2:PAD + 2 + TQ, 3 * c4:4 * c4],
    ], axis=-1).astype(bf16)
    xf = x_v[pl.ds(r0, TQ), :].astype(f32)
    x1 = xf + _dot(hs_in, w2_v[...])
    a = _dot(ot_scr[...].T.astype(bf16), wo_v[...])
    ln1 = _layernorm(x1).astype(bf16)
    nf = F // FC
    u_next = _dot(ln1, w3_v[:, 0:FC])
    bb = x1
    for c in range(nf):
        u = u_next
        if c + 1 < nf:
            u_next = _dot(ln1, w3_v[:, (c + 1) * FC:(c + 2) * FC])
        bb = bb + _dot(_gelu(u).astype(bf16), w4_v[c * FC:(c + 1) * FC, :])

    gate = jax.nn.sigmoid(jnp.sum(xf * gw_ref[...].astype(f32).reshape(1, D), axis=-1, keepdims=True))
    gb = (1.0 - gate) * bb
    gb_scr[...] = gb
    gate_scr[...] = gate
    o_ref[...] = (gate * a + gb).astype(o_ref.dtype)

    l_all = l_scr[...]
    safe = jnp.logical_and(jnp.min(l_all) >= L_MIN, jnp.max(l_all) <= L_MAX)

    @pl.when(jnp.logical_not(safe))
    def _():
        row_head = jax.lax.broadcasted_iota(jnp.int32, (128, TQ), 0) // DH

        def head(h, carry):
            g = h // HPG
            qg = qt_scr[pl.ds(pl.multiple_of(g * 128, 128), 128), :]
            w = jnp.where(row_head == h % HPG, qg, jnp.zeros_like(qg))
            s = _dot(k_scr[g], w)
            p = jnp.exp2(s - jnp.max(s, axis=0, keepdims=True))
            l = jnp.sum(p, axis=0, keepdims=True)
            pb = p.astype(bf16)
            r = pl.ds(pl.multiple_of(h * DH, DH), DH)
            o = jnp.zeros((DH, TQ), f32)
            for b in range(NB):
                o = o + _dot(vt_scr[b, r, :], pb[b * TQ:(b + 1) * TQ, :])
            ot_scr[r, :] = o / l
            return carry

        jax.lax.fori_loop(0, H, head, 0)
        a2 = _dot(ot_scr[...].T.astype(bf16), wo_v[...])
        o_ref[...] = (gate_scr[...] * a2 + gb_scr[...]).astype(o_ref.dtype)


@jax.jit
def pallas_gated_mix__mha_block__mixer_s_mlp__prompt_kernel(
    A_x: jax.Array,
    A_wqkv: jax.Array,
    A_wo: jax.Array,
    B_x: jax.Array,
    B_w1: jax.Array,
    B_w2: jax.Array,
    B_w3: jax.Array,
    B_w4: jax.Array,
    gate_w: jax.Array,
):
    ax = A_x.reshape(S, D)
    hbm = pl.BlockSpec(memory_space=pl.ANY)
    out = pl.pallas_call(
        _kernel,
        grid=(NB,),
        in_specs=[hbm] * 7 + [pl.BlockSpec((D,), lambda i: (0,))],
        out_specs=pl.BlockSpec((TQ, D), lambda i: (i, 0)),
        out_shape=jax.ShapeDtypeStruct((S, D), bf16),
        scratch_shapes=[
            pltpu.VMEM((S + PAD, D), bf16),
            pltpu.VMEM((D, 3 * D), bf16),
            pltpu.VMEM((D, D), bf16),
            pltpu.VMEM((D, D), bf16),
            pltpu.VMEM((D, D), bf16),
            pltpu.VMEM((D, F), bf16),
            pltpu.VMEM((F, D), bf16),
            pltpu.SemaphoreType.DMA((8,)),
            pltpu.SemaphoreType.DMA((NB,)),
            pltpu.VMEM((D, D), bf16),
            pltpu.VMEM((D, D), bf16),
            pltpu.VMEM((NG, S, 128), bf16),
            pltpu.VMEM((D, TQ), bf16),
            pltpu.VMEM((NB, D, TQ), bf16),
            pltpu.VMEM((D, TQ), f32),
            pltpu.VMEM((H, TQ), f32),
            pltpu.VMEM((H, TQ), f32),
            pltpu.VMEM((TQ, D), f32),
            pltpu.VMEM((TQ, 1), f32),
        ],
        compiler_params=pltpu.CompilerParams(
            dimension_semantics=("arbitrary",),
            vmem_limit_bytes=100 * 1024 * 1024),
    )(ax, A_wqkv, A_wo, B_w1, B_w2, B_w3, B_w4, gate_w)
    return out.reshape(1, S, D)
```
